```python
import jax
import jax.numpy as jnp

def _softmax(x, axis=-1):
    return jax.nn.softmax(x, axis=axis)
def _gelu(x):
    return jax.nn.gelu(x, approximate=True)
def _silu(x):
    return jax.nn.silu(x)
def _sigmoid(x):
    return jax.nn.sigmoid(x)
def _layernorm(x, axis=-1, eps=1e-5):
    m = jnp.mean(x, axis=axis, keepdims=True)
    v = jnp.var(x, axis=axis, keepdims=True)
    return (x - m) / jnp.sqrt(v + eps)
def _scatter_add(tgt, idx, src, axis=0):
    return tgt.at[idx].add(src)
def _segment_sum(src, seg, n):
    return jax.ops.segment_sum(src, seg, n)
class _Rng:
    def __init__(self, key):
        self._k = key
    def _next(self):
        self._k, sub = jax.random.split(self._k)
        return sub
    def normal(self, shape):
        return jax.random.normal(self._next(), shape, dtype=jnp.bfloat16)
    def randint(self, lo, hi, shape):
        return jax.random.randint(self._next(), shape, lo, hi, dtype=jnp.int32)
    def uniform(self, shape, lo=0.0, hi=1.0):
        return jax.random.uniform(self._next(), shape, jnp.bfloat16, lo, hi)
    def permutation(self, n):
        return jax.random.permutation(self._next(), n)


kernel_name = 'standalone__groupnorm__prompt'

def setup_inputs():
    _rng = _Rng(jax.random.key(int.from_bytes(__import__("os").urandom(4), "little")))
    _w = (lambda a: (lambda t: t.astype(jnp.bfloat16) if jnp.issubdtype(t.dtype, jnp.floating) else t)(jnp.asarray(a)))
    B = 2
    G = 32
    cpg = max(1, 1024 // G)
    C = G * cpg
    H, W = 32, 2048
    return {
        "x": _w((lambda *s: _rng.normal(s) * 0.05)(B, C, H, W)),
        "g": _w((lambda *s: _rng.normal(s) * 0.05)(C) + 1.0),
        "b": _w((lambda *s: _rng.normal(s) * 0.05)(C)),
    }

def reference(x, g, b):
    G = 32
    B, C, H, W = x.shape[0], x.shape[1], x.shape[2], x.shape[3]
    xr = x.reshape(B, G, C // G, H, W)
    mu = xr.mean(axis=(2, 3, 4), keepdims=True)
    var = ((xr - mu) ** 2).mean(axis=(2, 3, 4), keepdims=True)
    xn = (xr - mu) / jnp.sqrt(var + 1e-5)
    xn = xn.reshape(B, C, H, W)
    return xn * g[None, :, None, None] + b[None, :, None, None]
```

```python
import jax
import jax.numpy as jnp
from jax import lax
import jax.experimental.pallas as pl
import jax.experimental.pallas.tpu as pltpu

EPS = 1e-5
NUM_GROUPS = 32
PHASE_SIZES = (22, 21, 21)
CW = 1024
W0 = 2
TAIL_W = 2
RSPLIT = 7


@jax.jit
def pallas_standalone__groupnorm__prompt_kernel(
    x: jax.Array,
    g: jax.Array,
    b: jax.Array,
):
    B, C, H, W = x.shape
    G = NUM_GROUPS
    cpg = C // G
    NG = B * G
    S = 8
    CS = cpg // S
    assert sum(PHASE_SIZES) == NG
    NS = max(PHASE_SIZES)
    HH = H // 16
    J = W // CW
    NWR = CS * HH * J
    n_el = cpg * H * W
    starts = [0]
    for k in PHASE_SIZES:
        starts.append(starts[-1] + k)

    x5 = x.reshape(NG, S, CS, H, W)
    gb = jnp.stack([g, b]).astype(jnp.float32)

    def kernel(gb_ref, x_hbm, o_hbm, buf, rsem_a, rsem_b, wsem, wsem_tail):
        def rd_a(gi, slot):
            return pltpu.make_async_copy(
                x_hbm.at[gi, pl.ds(0, RSPLIT)], buf.at[slot, pl.ds(0, RSPLIT)], rsem_a.at[gi % 3])

        def rd_b(gi, slot):
            return pltpu.make_async_copy(
                x_hbm.at[gi, pl.ds(RSPLIT, S - RSPLIT)], buf.at[slot, pl.ds(RSPLIT, S - RSPLIT)],
                rsem_b.at[gi % 3])

        def start_read(gi, slot):
            rd_a(gi, slot).start()
            rd_b(gi, slot).start()

        def wr(gi, slot, u, sem):
            c = u // (HH * J)
            h = (u // J) % HH
            j = u % J
            return pltpu.make_async_copy(
                buf.at[slot, :, c, pl.ds(h * 16, 16), pl.ds(j * CW, CW)],
                o_hbm.at[gi, :, c, pl.ds(h * 16, 16), pl.ds(j * CW, CW)], sem)

        def start_write(gi, slot):
            for u in range(NWR):
                sem = wsem.at[slot] if u < NWR - TAIL_W else wsem_tail.at[slot]
                wr(gi, slot, u, sem).start()

        def wait_write_head(gi, slot):
            for u in range(NWR - TAIL_W):
                wr(gi, slot, u, wsem.at[slot]).wait()

        def wait_write_tail(gi, slot):
            for u in range(NWR - TAIL_W, NWR):
                wr(gi, slot, u, wsem_tail.at[slot]).wait()

        def compute(gi, slot):
            def load(ch):
                return buf[slot, ch // CS, ch % CS].astype(jnp.float32)

            def fold(v):
                r = v[0:8]
                for k in range(1, H // 8):
                    r = r + v[8 * k:8 * k + 8]
                return r

            def p1(ch, acc):
                return acc + fold(load(ch))
            acc = lax.fori_loop(0, cpg, p1, jnp.zeros((8, W), jnp.float32))
            mu = jnp.sum(acc, keepdims=True) * (1.0 / n_el)

            def p2(ch, acc):
                d = load(ch) - mu
                return acc + fold(d * d)
            acc = lax.fori_loop(0, cpg, p2, jnp.zeros((8, W), jnp.float32))
            var = jnp.sum(acc, keepdims=True) * (1.0 / n_el)
            rstd = lax.rsqrt(var + EPS)
            cbase = (gi % G) * cpg

            def p3(ch, c):
                a = rstd * gb_ref[0, cbase + ch]
                sh = gb_ref[1, cbase + ch] - mu * a
                buf[slot, ch // CS, ch % CS] = (load(ch) * a + sh).astype(buf.dtype)
                return c
            lax.fori_loop(0, cpg, p3, 0)

        start_read(0, 0)
        start_read(1, 1)

        def body(gi, carry):
            p0 = jnp.int32(0)
            p1_ = jnp.int32(starts[1])
            for st, en in zip(starts[1:-1], starts[2:]):
                p0 = jnp.where(gi >= st, st, p0)
                p1_ = jnp.where(gi >= st, en, p1_)
            slot = gi - p0
            is_last = gi == p1_ - 1
            rd_a(gi, slot).wait()

            @pl.when(is_last)
            def _():
                for k in range(W0):
                    start_write(p0 + k, k)
            rd_b(gi, slot).wait()

            @pl.when(gi + 2 < p1_)
            def _():
                start_read(gi + 2, slot + 2)
            compute(gi, slot)

            @pl.when(is_last)
            def _():
                K = p1_ - p0

                def wbody(k, c):
                    wait_write_head(p0 + k - W0, k - W0)
                    wait_write_tail(p0 + k - W0, k - W0)
                    start_write(p0 + k, k)
                    return c
                lax.fori_loop(W0, K, wbody, 0)
                for k in range(W0 - 1):
                    wait_write_head(p0 + K - W0 + k, K - W0 + k)
                    wait_write_tail(p0 + K - W0 + k, K - W0 + k)
                wait_write_head(p0 + K - 1, K - 1)

                @pl.when(p1_ < NG)
                def _():
                    start_read(p1_, 0)
                    start_read(p1_ + 1, 1)
                wait_write_tail(p0 + K - 1, K - 1)
            return carry
        lax.fori_loop(0, NG, body, 0)

    out = pl.pallas_call(
        kernel,
        in_specs=[pl.BlockSpec(memory_space=pltpu.SMEM), pl.BlockSpec(memory_space=pl.ANY)],
        out_specs=pl.BlockSpec(memory_space=pl.ANY),
        out_shape=jax.ShapeDtypeStruct(x5.shape, x.dtype),
        scratch_shapes=[
            pltpu.VMEM((NS, S, CS, H, W), x.dtype),
            pltpu.SemaphoreType.DMA((3,)),
            pltpu.SemaphoreType.DMA((3,)),
            pltpu.SemaphoreType.DMA((NS,)),
            pltpu.SemaphoreType.DMA((NS,)),
        ],
        compiler_params=pltpu.CompilerParams(vmem_limit_bytes=NS * 4 * 1024 * 1024 + 8 * 1024 * 1024),
    )(gb, x5)
    return out.reshape(x.shape)
```

```python
import functools
import jax
import jax.numpy as jnp
from jax import lax
from jax.experimental import pallas as pl
from jax.experimental.pallas import tpu as pltpu

EPS = 1e-5
NUM_GROUPS = 32


def _make_kernel(phase_sizes=(11, 11, 10), D=16, DH=4, RW_LEAD=3, TAIL_W=1, wcw=2048, rcw=1024, do_compute=True,
                unroll=1, NL=7):
    @jax.jit
    def fn(x, g, b):
        B, C, H, W = x.shape
        G = NUM_GROUPS
        cpg = C // G
        GPW = 2
        S = 8
        CS = GPW * cpg // S
        SPG = S // GPW
        NW = B * G // GPW
        assert sum(phase_sizes) == NW
        NS = max(phase_sizes)
        R = H // 8
        RJ = W // rcw
        KS = R * RJ
        SPW = CS * KS
        WJ = W // wcw
        NWR = CS * R * WJ
        n_el = cpg * H * W
        assert D % KS == 0 or KS % D == 0

        x6 = x.reshape(NW, S, CS, H, W)
        gb = jnp.stack([g, b]).astype(jnp.float32)

        def kernel(gb_ref, x_hbm, o_hbm, buf, lsem, hsem, wsem, tsem):
            def step_idx(i):
                slot = i // SPW
                u = i % SPW
                c = u // KS
                r = (u // RJ) % R
                j = u % RJ
                if isinstance(i, int):
                    return slot, c, pl.ds(r * 8, 8), pl.ds(j * rcw, rcw)
                return slot, c, pl.ds(pl.multiple_of(r * 8, 8), 8), pl.ds(pl.multiple_of(j * rcw, rcw), rcw)

            def low(w0, i):
                slot, c, rs, cs = step_idx(i)
                return pltpu.make_async_copy(
                    x_hbm.at[w0 + slot, pl.ds(0, NL), c, rs, cs], buf.at[slot, pl.ds(0, NL), c, rs, cs], lsem.at[i % D])

            def high(w0, i):
                slot, c, rs, cs = step_idx(i)
                return pltpu.make_async_copy(
                    x_hbm.at[w0 + slot, pl.ds(NL, S - NL), c, rs, cs], buf.at[slot, pl.ds(NL, S - NL), c, rs, cs],
                    hsem.at[slot])

            def wait_high_window(w0, slot):
                pltpu.make_async_copy(
                    x_hbm.at[w0 + slot, pl.ds(NL, S - NL)], buf.at[slot, pl.ds(NL, S - NL)], hsem.at[slot]).wait()

            def wr(w0, slot, u, sem):
                c = u // (R * WJ)
                r = (u // WJ) % R
                j = u % WJ
                return pltpu.make_async_copy(
                    buf.at[slot, :, c, pl.ds(r * 8, 8), pl.ds(j * wcw, wcw)],
                    o_hbm.at[w0 + slot, :, c, pl.ds(r * 8, 8), pl.ds(j * wcw, wcw)], sem)

            def start_write(w0, slot, split_tail):
                for u in range(NWR):
                    sem = tsem.at[0] if (split_tail and u >= NWR - TAIL_W) else wsem.at[slot]
                    wr(w0, slot, u, sem).start()

            def wait_write_full(w0, slot):
                pltpu.make_async_copy(buf.at[slot], o_hbm.at[w0 + slot], wsem.at[slot]).wait()

            def compute_group(w, slot, q, hook):
                def ref_of(ch):
                    return buf.at[slot, q * SPG + ch // CS, ch % CS]

                def fold(v):
                    r = v[0:8]
                    for k in range(1, H // 8):
                        r = r + v[8 * k:8 * k + 8]
                    return r

                def p1(ch, acc):
                    hook(ch)
                    return acc + fold(ref_of(ch)[...].astype(jnp.float32))
                acc = lax.fori_loop(0, cpg, p1, jnp.zeros((8, W), jnp.float32), unroll=unroll)
                mu = jnp.sum(acc, keepdims=True) * (1.0 / n_el)

                def p2(ch, acc):
                    hook(cpg + ch)
                    d = ref_of(ch)[...].astype(jnp.float32) - mu
                    return acc + fold(d * d)
                acc = lax.fori_loop(0, cpg, p2, jnp.zeros((8, W), jnp.float32), unroll=unroll)
                var = jnp.sum(acc, keepdims=True) * (1.0 / n_el)
                rstd = lax.rsqrt(var + EPS)
                cbase = ((w * GPW + q) % G) * cpg

                def p3(ch, c):
                    hook(2 * cpg + ch)
                    a = rstd * gb_ref[0, cbase + ch]
                    sh = gb_ref[1, cbase + ch] - mu * a
                    r = ref_of(ch)
                    r[...] = (r[...].astype(jnp.float32) * a + sh).astype(buf.dtype)
                    return c
                lax.fori_loop(0, cpg, p3, 0, unroll=unroll)

            def start_read_phase(w0):
                for i in range(DH):
                    high(w0, i).start(priority=0)
                for i in range(D):
                    low(w0, i).start(priority=1)

            def phase(w0, K, is_last_phase):
                N = K * SPW

                def pace(i):
                    low(w0, i).wait()
                    high(w0, i + DH).start(priority=0)
                    low(w0, i + D).start(priority=1)

                def pace_loop(lo, hi):
                    def body(i, c):
                        pace(i)
                        return c
                    lax.fori_loop(lo, hi, body, 0)

                pace_loop(0, SPW)
                wait_high_window(w0, 0)
                pos = SPW
                if do_compute:
                    def cg(q, c):
                        compute_group(w0, 0, q, lambda k: pace(SPW + q * 3 * cpg + k))
                        return c
                    lax.fori_loop(0, GPW, cg, 0)
                    pos = SPW + GPW * 3 * cpg
                pace_loop(pos, N - D)
                for t in range(D):
                    i = N - D + t
                    low(w0, i).wait()
                    if t + DH < D:
                        high(w0, i + DH).start(priority=0)
                    if t == D - 1 - RW_LEAD:
                        start_write(w0, 0, False)

                def wbody(slot, c):
                    wait_high_window(w0, slot)
                    if do_compute:
                        def cg(q, c):
                            compute_group(w0 + slot, slot, q, lambda k: None)
                            return c
                        lax.fori_loop(0, GPW, cg, 0)

                    @pl.when(slot < K - 1)
                    def _():
                        start_write(w0, slot, False)

                    @pl.when(slot == K - 1)
                    def _():
                        start_write(w0, slot, True)
                    return c
                lax.fori_loop(1, K, wbody, 0)

                def wwait(slot, c):
                    wait_write_full(w0, slot)
                    return c
                lax.fori_loop(0, K - 1, wwait, 0)
                for u in range(NWR - TAIL_W):
                    wr(w0, K - 1, u, wsem.at[K - 1]).wait()

                @pl.when(jnp.logical_not(is_last_phase))
                def _():
                    start_read_phase(w0 + K)
                for u in range(NWR - TAIL_W, NWR):
                    wr(w0, K - 1, u, tsem.at[0]).wait()

            start_read_phase(0)
            starts = [0]
            for k in phase_sizes:
                starts.append(starts[-1] + k)

            def pbody(p, c):
                w0 = jnp.int32(0)
                K = jnp.int32(phase_sizes[0])
                for pp in range(1, len(phase_sizes)):
                    w0 = jnp.where(p == pp, starts[pp], w0)
                    K = jnp.where(p == pp, phase_sizes[pp], K)
                phase(w0, K, p == len(phase_sizes) - 1)
                return c
            lax.fori_loop(0, len(phase_sizes), pbody, 0)

        out = pl.pallas_call(
            kernel,
            in_specs=[pl.BlockSpec(memory_space=pltpu.SMEM), pl.BlockSpec(memory_space=pl.ANY)],
            out_specs=pl.BlockSpec(memory_space=pl.ANY),
            out_shape=jax.ShapeDtypeStruct(x6.shape, x.dtype),
            scratch_shapes=[
                pltpu.VMEM((NS, S, CS, H, W), x.dtype),
                pltpu.SemaphoreType.DMA((D,)),
                pltpu.SemaphoreType.DMA((NS,)),
                pltpu.SemaphoreType.DMA((NS,)),
                pltpu.SemaphoreType.DMA((1,)),
            ],
            compiler_params=pltpu.CompilerParams(vmem_limit_bytes=NS * 8 * 1024 * 1024 + 8 * 1024 * 1024),
        )(gb, x6)
        return out.reshape(x.shape)
    return fn


pallas_standalone__groupnorm__prompt_kernel = _make_kernel()
```

```python
import jax
import jax.numpy as jnp
from jax import lax
import jax.experimental.pallas as pl
import jax.experimental.pallas.tpu as pltpu

EPS = 1e-5
NUM_GROUPS = 32


def _shr(v, n):
    return v >> n if isinstance(v, int) else lax.shift_right_logical(v, jnp.int32(n))


def _and(v, m):
    return v & m if isinstance(v, int) else lax.bitwise_and(v, jnp.int32(m))


def _sel(p, vals):
    r = jnp.int32(vals[0])
    for i in range(1, len(vals)):
        r = jnp.where(p == i, jnp.int32(vals[i]), r)
    return r


def _make_kernel(D=16, DH=4, RW_LEAD=3, TAIL=1, wcw=1024, do_compute=True, nobounds=True, AW=256, CU=8):
    @jax.jit
    def fn(x, g, b):
        B, C, H, W = x.shape
        G = NUM_GROUPS
        cpg = C // G
        NG = B * G
        assert (B, C, H, W) == (2, 1024, 32, 2048)
        RS = 8
        SPC = H // RS
        CPS = 8
        SL = CPS * SPC
        NSTR = B * C // CPS
        S = 8
        SHIFT = 2
        NWIN = NSTR // S
        V = NWIN - 1
        RING = 11
        HW = W // 2
        SPW = SL * 2
        n_el = cpg * H * W
        WJ = W // wcw
        KR0 = (0, 11, 21)
        NWR = (11, 10, 10)
        GA = (0, 22, 42)
        LEAD = (4, 2, 2)
        NM = (18, 18, 20)
        KA = (0, 10, 20)
        NKW = (10, 10, 11)
        NP = 3

        x4 = x.reshape(NSTR, SL, RS, W)
        g2 = g.reshape(8, C // 8)
        b2 = b.reshape(8, C // 8)

        def kernel(x_hbm, g_hbm, b_hbm, o_hbm, buf, gb_bf, gb_f32, gb_s, lsem, hsem, wsem, tsem, psem):
            def pos_of(k):
                if isinstance(k, int):
                    return k % RING
                return k - jnp.where(k >= 2 * RING, 2 * RING, jnp.where(k >= RING, RING, 0))

            def piece(u):
                if isinstance(u, int):
                    return u >> 1, pl.ds((u & 1) * HW, HW)
                return _shr(u, 1), pl.ds(pl.multiple_of(_and(u, 1) * HW, HW), HW)

            def rd(n0, v0, ns, u, sem):
                sl, cs = piece(u)
                return pltpu.make_async_copy(
                    x_hbm.at[pl.ds(n0, ns), sl, :, cs], buf.at[pl.ds(v0, ns), sl, :, cs], sem)

            def start_low(kr0, j):
                k = kr0 + _shr(j, 6)
                rd(k * S + SHIFT, pos_of(k) * S, S - 1, _and(j, SPW - 1), lsem.at[_and(j, D - 1)]).start(priority=1)

            def start_high(kr0, j):
                k = kr0 + _shr(j, 6)
                rd(k * S + SHIFT + S - 1, pos_of(k) * S + S - 1, 1, _and(j, SPW - 1),
                   hsem.at[_and(j, 2 * DH - 1)]).start(priority=0)

            def start_low_v(j):
                sem = lsem.at[_and(j, D - 1)]
                rd(V * S + SHIFT, RING * S, S - SHIFT, j, sem).start(priority=1)
                rd(0, RING * S + S - SHIFT, SHIFT - 1, j, sem).start(priority=1)

            def start_high_v(j):
                rd(SHIFT - 1, RING * S + S - 1, 1, j, hsem.at[_and(j, 2 * DH - 1)]).start(priority=0)

            def wait_step(j):
                rd(0, 0, S - 1, 0, lsem.at[_and(j, D - 1)]).wait()
                rd(0, 0, 1, 0, hsem.at[_and(j, 2 * DH - 1)]).wait()

            def read_prologue(kr0):
                for j in range(DH):
                    start_high(kr0, j)
                for j in range(D):
                    start_low(kr0, j)

            def wr(n0, v0, ns, sl, jj, sem):
                cs = pl.ds(jj * wcw, wcw)
                return pltpu.make_async_copy(
                    buf.at[pl.ds(v0, ns), sl, :, cs], o_hbm.at[pl.ds(n0, ns), sl, :, cs], sem)

            def issue_slabs(start_fn, pos, lo, hi, sem):
                def body(sl, c):
                    for jj in range(WJ):
                        start_fn(sl, jj, sem)
                    return c
                lax.fori_loop(lo, hi, body, 0)

            def issue_chunk_generic(start_fn, pos, half):
                lo = half * (SL // 2)
                hi_head = lo + SL // 2 - half * TAIL
                issue_slabs(start_fn, pos, lo, hi_head, wsem.at[pos])
                issue_slabs(start_fn, pos, hi_head, lo + SL // 2, tsem.at[pos])

            def issue_chunk(cid):
                k = _shr(cid, 1)
                pos = pos_of(k)
                issue_chunk_generic(
                    lambda sl, jj, sem: wr(k * S + SHIFT, pos * S, S, sl, jj, sem).start(), pos, _and(cid, 1))

            def issue_chunk_v(half):
                def st(sl, jj, sem):
                    wr(V * S + SHIFT, RING * S, S - SHIFT, sl, jj, sem).start()
                    wr(0, RING * S + S - SHIFT, SHIFT, sl, jj, sem).start()
                issue_chunk_generic(st, RING, half)

            def wait_head(pos):
                r = buf.at[pl.ds(pos * S, S), pl.ds(0, SL - TAIL)]
                pltpu.make_async_copy(r, r, wsem.at[pos]).wait()

            def wait_tail(pos):
                r = buf.at[pl.ds(pos * S, S), pl.ds(SL - TAIL, TAIL)]
                pltpu.make_async_copy(r, r, tsem.at[pos]).wait()

            def tree(parts):
                while len(parts) > 1:
                    parts = [parts[i] + parts[i + 1] for i in range(0, len(parts), 2)]
                return parts[0]

            def compute_group(gi, hook, cu):
                def vstream(s):
                    n = _and(gi * 4 + s - SHIFT, NSTR - 1)
                    k = _shr(n, 3)
                    return jnp.where(k == V, RING, pos_of(k)) * S + _and(n, S - 1)
                nit = cpg // cu
                ips = CPS // cu

                def refs(it):
                    if ips == 1:
                        base = buf.at[vstream(it)]
                        return [base.at[pl.ds(c * SPC, SPC)] for c in range(cu)]
                    sh = ips.bit_length() - 1
                    base = buf.at[vstream(_shr(it, sh)), pl.ds(_and(it, ips - 1) * (cu * SPC), cu * SPC)]
                    return [base.at[pl.ds(c * SPC, SPC)] for c in range(cu)]

                def red(r, f):
                    outs = []
                    for k in range(SPC):
                        v = f(r[k].astype(jnp.float32))
                        outs.append(tree([v[:, j * AW:(j + 1) * AW] for j in range(W // AW)]))
                    return tree(outs)

                def p1(it, acc):
                    for c, r in enumerate(refs(it)):
                        hook(it * cu + c)
                        acc = acc + red(r, lambda v: v)
                    return acc
                acc = lax.fori_loop(0, nit, p1, jnp.zeros((RS, AW), jnp.float32))
                mu = jnp.sum(acc, keepdims=True) * (1.0 / n_el)

                def sq(v):
                    d = v - mu
                    return d * d

                def p2(it, acc):
                    for c, r in enumerate(refs(it)):
                        hook(cpg + it * cu + c)
                        acc = acc + red(r, sq)
                    return acc
                acc = lax.fori_loop(0, nit, p2, jnp.zeros((RS, AW), jnp.float32))
                var = jnp.sum(acc, keepdims=True) * (1.0 / n_el)
                rstd = lax.rsqrt(var + EPS)
                cb = _and(gi, G - 1) * cpg
                crow = _shr(cb, 7)
                ccol = _and(cb, 127)

                def p3(it, carry):
                    for c, r in enumerate(refs(it)):
                        hook(2 * cpg + it * cu + c)
                        ch = ccol + it * cu + c
                        a = rstd * gb_s[crow, ch]
                        sh = gb_s[8 + crow, ch] - mu * a
                        r[...] = (r[...].astype(jnp.float32) * a + sh).astype(buf.dtype)
                    return carry
                lax.fori_loop(0, nit, p3, 0)

            for j in range(DH):
                start_high_v(j)
            for j in range(D):
                start_low_v(j)
            cg = pltpu.make_async_copy(g_hbm, gb_bf.at[0], psem.at[0])
            cb_ = pltpu.make_async_copy(b_hbm, gb_bf.at[1], psem.at[1])
            cg.start()
            cb_.start()

            def va(j, c):
                wait_step(j)
                start_high_v(j + DH)
                start_low_v(j + D)
                return c
            lax.fori_loop(0, 8, va, 0)
            cg.wait()
            cb_.wait()
            gb_f32[0:8, :] = gb_bf[0].astype(jnp.float32)
            gb_f32[8:16, :] = gb_bf[1].astype(jnp.float32)
            cs_ = pltpu.make_async_copy(gb_f32, gb_s, psem.at[2])
            cs_.start()
            lax.fori_loop(8, SPW - D, va, 0)
            cs_.wait()

            def vb(j, c):
                wait_step(j)
                start_high_v(j + DH)
                start_low(0, j + D - SPW)
                return c
            lax.fori_loop(SPW - D, SPW - DH, vb, 0)
            for j in range(SPW - DH, SPW):
                wait_step(j)
                start_high(0, j + DH - SPW)
                start_low(0, j + D - SPW)

            def phase(p, carry):
                kr0 = _sel(p, KR0)
                nsteps = _sel(p, NWR) * SPW
                ga = _sel(p, GA)
                lead = _sel(p, LEAD)
                ka = _sel(p, KA)

                def pace(j):
                    wait_step(j)
                    start_high(kr0, j + DH)
                    start_low(kr0, j + D)

                def pace_loop(lo, hi):
                    def body(j, c):
                        pace(j)
                        return c
                    lax.fori_loop(lo, hi, body, 0)

                pace_loop(0, SPW)
                pos = SPW
                if do_compute:
                    def cgl(q, c):
                        compute_group(ga + q, lambda k: pace(SPW + q * (3 * cpg) + k), 1)
                        return c
                    lax.fori_loop(0, lead, cgl, 0)
                    pos = SPW + lead * (3 * cpg)
                pace_loop(pos, nsteps - D)
                for t in range(D):
                    j = nsteps - D + t
                    wait_step(t)
                    if t + DH < D:
                        start_high(kr0, j + DH)
                    if t == D - 1 - RW_LEAD:
                        issue_chunk(2 * ka)
                issue_chunk(2 * ka + 1)

                def wbody(m, c):
                    if do_compute:
                        compute_group(ga + lead + m, lambda k: None, CU)
                    issue_chunk(2 * ka + 2 + m)
                    return c
                lax.fori_loop(0, _sel(p, NM), wbody, 0)

                @pl.when(p == NP - 1)
                def _():
                    issue_chunk_v(0)
                    issue_chunk_v(1)

                k_last = ka + _sel(p, NKW) - 1

                def wwait(k, c):
                    wait_head(pos_of(k))
                    wait_tail(pos_of(k))
                    return c
                lax.fori_loop(ka, k_last, wwait, 0)
                wait_head(pos_of(k_last))

                @pl.when(p < NP - 1)
                def _():
                    read_prologue(kr0 + _sel(p, NWR))
                wait_tail(pos_of(k_last))
                return carry
            lax.fori_loop(0, NP, phase, 0)
            wait_head(RING)
            wait_tail(RING)

        out = pl.pallas_call(
            kernel,
            in_specs=[pl.BlockSpec(memory_space=pl.ANY)] * 3,
            out_specs=pl.BlockSpec(memory_space=pl.ANY),
            out_shape=jax.ShapeDtypeStruct(x4.shape, x.dtype),
            scratch_shapes=[
                pltpu.VMEM(((RING + 1) * S, SL, RS, W), x.dtype),
                pltpu.VMEM((2, 8, C // 8), g.dtype),
                pltpu.VMEM((16, C // 8), jnp.float32),
                pltpu.SMEM((16, C // 8), jnp.float32),
                pltpu.SemaphoreType.DMA((D,)),
                pltpu.SemaphoreType.DMA((2 * DH,)),
                pltpu.SemaphoreType.DMA((RING + 1,)),
                pltpu.SemaphoreType.DMA((RING + 1,)),
                pltpu.SemaphoreType.DMA((3,)),
            ],
            compiler_params=pltpu.CompilerParams(
                vmem_limit_bytes=(RING + 1) * 8 * 1024 * 1024 + 8 * 1024 * 1024,
                disable_bounds_checks=nobounds),
        )(x4, g2, b2)
        return out.reshape(x.shape)
    return fn


pallas_standalone__groupnorm__prompt_kernel = _make_kernel()
```

```python
import jax
import jax.numpy as jnp
from jax import lax
import jax.experimental.pallas as pl
import jax.experimental.pallas.tpu as pltpu

EPS = 1e-5
NUM_GROUPS = 32


def _shr(v, n):
    return v >> n if isinstance(v, int) else lax.shift_right_logical(v, jnp.int32(n))


def _and(v, m):
    return v & m if isinstance(v, int) else lax.bitwise_and(v, jnp.int32(m))


def _sel(p, vals):
    r = jnp.int32(vals[0])
    for i in range(1, len(vals)):
        r = jnp.where(p == i, jnp.int32(vals[i]), r)
    return r


def _make_kernel(D=16, DH=8, RW_LEAD=7, TJ=4, TW=2, wcw=1024, rcw=256, do_compute=True, nobounds=True,
                AW=256, CU=8, HK=2):
    @jax.jit
    def fn(x, g, b):
        B, C, H, W = x.shape
        assert (B, C, H, W) == (2, 1024, 32, 2048)
        G = NUM_GROUPS
        cpg = C // G
        RS = 8
        SPC = H // RS
        CPS = 8
        SH = CPS * SPC // 2
        NSTR = B * C // CPS
        S = 8
        SHIFT = 2
        V = NSTR // S - 1
        RING = 11
        RJ = W // rcw
        SPW = SH * RJ
        LSPW = SPW.bit_length() - 1
        LRJ = RJ.bit_length() - 1
        NSL = 3 * cpg * HK
        WJ = W // wcw
        tcw = W // TJ
        NHS = 2 * DH
        n_el = cpg * H * W
        KR0 = (0, 11, 21)
        NWR = (11, 10, 10)
        GA = (0, 22, 42)
        LEAD = (4, 2, 2)
        NM = (18, 18, 20)
        KA = (0, 10, 20)
        NKW = (10, 10, 11)
        NP = 3
        assert SPW % D == 0 and SPW % NHS == 0 and D % NHS == 0 and DH <= D and RW_LEAD < D
        assert all(SPW + l * NSL <= n * SPW - D for l, n in zip(LEAD, NWR)) and 2 * NSL >= SPW

        x5 = x.reshape(NSTR, 2, SH, RS, W)
        g2 = g.reshape(8, C // 8)
        b2 = b.reshape(8, C // 8)

        def kernel(x_hbm, g_hbm, b_hbm, o_hbm, buf, gb_bf, gb_f32, gb_s, vsem):
            pl.run_scoped(
                lambda *sems: body(x_hbm, g_hbm, b_hbm, o_hbm, buf, gb_bf, gb_f32, gb_s, vsem, *sems),
                pltpu.SemaphoreType.DMA((D,)),
                pltpu.SemaphoreType.DMA((NHS,)),
                pltpu.SemaphoreType.DMA((2 * RING,)),
                pltpu.SemaphoreType.DMA((TJ * RING,)),
                pltpu.SemaphoreType.DMA((3,)))
            for n0, v0, ns in parts_v:
                pltpu.make_async_copy(buf.at[pl.ds(v0, ns)], o_hbm.at[pl.ds(n0, ns)], vsem.at[0]).wait()

        parts_v = [(V * S + SHIFT, RING * S, S - SHIFT), (0, RING * S + S - SHIFT, SHIFT)]

        def body(x_hbm, g_hbm, b_hbm, o_hbm, buf, gb_bf, gb_f32, gb_s, vsem, lsem, hsem, wsem, tsem, psem):
            def pos_of(k):
                if isinstance(k, int):
                    return k % RING
                return k - jnp.where(k >= 2 * RING, 2 * RING, jnp.where(k >= RING, RING, 0))

            def rd(n0, v0, ns, u, sem):
                sl = _shr(u, LRJ)
                c0 = _and(u, RJ - 1) * rcw
                cs = pl.ds(c0 if isinstance(c0, int) else pl.multiple_of(c0, rcw), rcw)
                return pltpu.make_async_copy(
                    x_hbm.at[pl.ds(n0, ns), :, sl, :, cs], buf.at[pl.ds(v0, ns), :, sl, :, cs], sem)

            def low(kr0, j):
                k = kr0 + _shr(j, LSPW)
                return [rd(k * S + SHIFT, pos_of(k) * S, S - 1, _and(j, SPW - 1), lsem.at[_and(j, D - 1)])]

            def high(kr0, j):
                k = kr0 + _shr(j, LSPW)
                return [rd(k * S + SHIFT + S - 1, pos_of(k) * S + S - 1, 1, _and(j, SPW - 1),
                           hsem.at[_and(j, NHS - 1)])]

            def low_v(j):
                sem = lsem.at[_and(j, D - 1)]
                return [rd(V * S + SHIFT, RING * S, S - SHIFT, j, sem),
                        rd(0, RING * S + S - SHIFT, SHIFT - 1, j, sem)]

            def high_v(j):
                return [rd(SHIFT - 1, RING * S + S - 1, 1, j, hsem.at[_and(j, NHS - 1)])]

            def start(copies, priority):
                for c in copies:
                    c.start(priority=priority)

            def wait(copies):
                for c in copies:
                    c.wait()

            def read_prologue(kr0):
                for j in range(DH):
                    start(high(kr0, j), 0)
                for j in range(D):
                    start(low(kr0, j), 1)

            def wr(parts, half, sl, cs, sem):
                return [pltpu.make_async_copy(buf.at[pl.ds(v0, ns), half, sl, :, cs],
                                              o_hbm.at[pl.ds(n0, ns), half, sl, :, cs], sem)
                        for n0, v0, ns in parts]

            def parts_of(k, pos):
                return [(k * S + SHIFT, pos * S, S)]

            def issue_chunk_of(parts, pos, half):
                def body(sl, c):
                    for jj in range(WJ):
                        start(wr(parts, half, sl, pl.ds(jj * wcw, wcw), wsem.at[2 * pos + half]), 0)
                    return c
                lax.fori_loop(0, SH - half, body, 0)

                def tail():
                    for t in range(TJ):
                        start(wr(parts, 1, SH - 1, pl.ds(t * tcw, tcw), tsem.at[TJ * pos + t]), 0)
                if isinstance(half, int):
                    if half == 1:
                        tail()
                else:
                    pl.when(half == 1)(tail)

            def issue_chunk(cid):
                k = _shr(cid, 1)
                pos = pos_of(k)
                issue_chunk_of(parts_of(k, pos), pos, _and(cid, 1))

            def wait_head(parts, pos):
                wait(wr(parts, 0, pl.ds(0, SH), pl.ds(0, W), wsem.at[2 * pos]))
                wait(wr(parts, 1, pl.ds(0, SH - 1), pl.ds(0, W), wsem.at[2 * pos + 1]))

            def wait_tail(parts, pos, lo, hi):
                for t in range(lo, hi):
                    wait(wr(parts, 1, SH - 1, pl.ds(t * tcw, tcw), tsem.at[TJ * pos + t]))

            def tree(parts):
                while len(parts) > 1:
                    parts = [parts[i] + parts[i + 1] for i in range(0, len(parts), 2)]
                return parts[0]

            def compute_group(gi, hook, cu):
                def vstream(s):
                    n = _and(gi * 4 + s - SHIFT, NSTR - 1)
                    k = _shr(n, 3)
                    return jnp.where(k == V, RING, pos_of(k)) * S + _and(n, S - 1)
                nit = cpg // cu
                ips = CPS // cu

                def refs(it):
                    if ips == 1:
                        base = buf.at[vstream(it)]
                        return [base.at[c // 4, pl.ds((c % 4) * SPC, SPC)] for c in range(cu)]
                    sh = ips.bit_length() - 1
                    base = buf.at[vstream(_shr(it, sh)), _and(_shr(it, sh - 1), 1),
                                  pl.ds(_and(it, ips // 2 - 1) * (cu * SPC), cu * SPC)]
                    return [base.at[pl.ds(c * SPC, SPC)] for c in range(cu)]

                def red(r, f, hk):
                    outs = []
                    for k in range(SPC):
                        if k % (SPC // HK) == 0:
                            hook(hk * HK + k // (SPC // HK))
                        v = f(r[k].astype(jnp.float32))
                        outs.append(tree([v[:, j * AW:(j + 1) * AW] for j in range(W // AW)]))
                    return tree(outs)

                def p1(it, acc):
                    for c, r in enumerate(refs(it)):
                        acc = acc + red(r, lambda v: v, it * cu + c)
                    return acc
                acc = lax.fori_loop(0, nit, p1, jnp.zeros((RS, AW), jnp.float32))
                mu = jnp.sum(acc, keepdims=True) * (1.0 / n_el)

                def sq(v):
                    d = v - mu
                    return d * d

                def p2(it, acc):
                    for c, r in enumerate(refs(it)):
                        acc = acc + red(r, sq, cpg + it * cu + c)
                    return acc
                acc = lax.fori_loop(0, nit, p2, jnp.zeros((RS, AW), jnp.float32))
                var = jnp.sum(acc, keepdims=True) * (1.0 / n_el)
                rstd = lax.rsqrt(var + EPS)
                cb = _and(gi, G - 1) * cpg
                crow = _shr(cb, 7)
                ccol = _and(cb, 127)

                def p3(it, carry):
                    for c, r in enumerate(refs(it)):
                        ch = ccol + it * cu + c
                        a = rstd * gb_s[crow, ch]
                        sh = gb_s[8 + crow, ch] - mu * a
                        for hh in range(HK):
                            hook((2 * cpg + it * cu + c) * HK + hh)
                            rr = r.at[pl.ds(hh * (SPC // HK), SPC // HK)]
                            rr[...] = (rr[...].astype(jnp.float32) * a + sh).astype(buf.dtype)
                    return carry
                lax.fori_loop(0, nit, p3, 0)

            for j in range(DH):
                start(high_v(j), 0)
            for j in range(D):
                start(low_v(j), 1)
            cp_g = pltpu.make_async_copy(g_hbm, gb_bf.at[0], psem.at[0])
            cp_b = pltpu.make_async_copy(b_hbm, gb_bf.at[1], psem.at[1])
            cp_g.start()
            cp_b.start()

            def va(j, c):
                wait(low_v(j))
                wait(high_v(j))
                start(high_v(j + DH), 0)
                start(low_v(j + D), 1)
                return c
            lax.fori_loop(0, 16, va, 0)
            cp_g.wait()
            cp_b.wait()
            gb_f32[0:8, :] = gb_bf[0].astype(jnp.float32)
            gb_f32[8:16, :] = gb_bf[1].astype(jnp.float32)
            cp_s = pltpu.make_async_copy(gb_f32, gb_s, psem.at[2])
            cp_s.start()
            lax.fori_loop(16, SPW - D, va, 0)
            cp_s.wait()
            for j in range(SPW - D, SPW):
                wait(low_v(j))
                wait(high_v(j))
                start(high_v(j + DH) if j + DH < SPW else high(0, j + DH - SPW), 0)
                start(low(0, j + D - SPW), 1)

            def phase(p, carry):
                kr0 = _sel(p, KR0)
                nsteps = _sel(p, NWR) * SPW
                ga = _sel(p, GA)
                lead = _sel(p, LEAD)
                ka = _sel(p, KA)

                def pace(j):
                    wait(low(kr0, j))
                    wait(high(kr0, j))
                    start(high(kr0, j + DH), 0)
                    start(low(kr0, j + D), 1)

                def pace_loop(lo, hi):
                    def body(j, c):
                        pace(j)
                        return c
                    lax.fori_loop(lo, hi, body, 0)

                pace_loop(0, SPW)
                pos = SPW
                if do_compute:
                    def cgl(q, c):
                        compute_group(ga + q, lambda k: pace(SPW + q * NSL + k), 1)
                        return c
                    lax.fori_loop(0, lead, cgl, 0)
                    pos = SPW + lead * NSL
                pace_loop(pos, nsteps - D)
                for t in range(D):
                    j = nsteps - D + t
                    wait(low(kr0, j))
                    wait(high(kr0, j))
                    if t + DH < D:
                        start(high(kr0, j + DH), 0)
                    if t == D - 1 - RW_LEAD:
                        issue_chunk(2 * ka)
                issue_chunk(2 * ka + 1)

                def wbody(m, c):
                    if do_compute:
                        compute_group(ga + lead + m, lambda k: None, CU)
                    issue_chunk(2 * ka + 2 + m)
                    return c
                lax.fori_loop(0, _sel(p, NM), wbody, 0)

                @pl.when(p == NP - 1)
                def _():
                    for half in range(2):
                        def vbody(sl, c):
                            for jj in range(WJ):
                                start(wr(parts_v, half, sl, pl.ds(jj * wcw, wcw), vsem.at[0]), 0)
                            return c
                        lax.fori_loop(0, SH, vbody, 0)

                k_last = ka + _sel(p, NKW) - 1

                def wwait(k, c):
                    wait_head(parts_of(k, pos_of(k)), pos_of(k))
                    wait_tail(parts_of(k, pos_of(k)), pos_of(k), 0, TJ)
                    return c
                lax.fori_loop(ka, k_last, wwait, 0)
                p_last = pos_of(k_last)
                wait_head(parts_of(k_last, p_last), p_last)
                wait_tail(parts_of(k_last, p_last), p_last, 0, TW)

                @pl.when(p < NP - 1)
                def _():
                    read_prologue(kr0 + _sel(p, NWR))
                wait_tail(parts_of(k_last, p_last), p_last, TW, TJ)
                return carry
            lax.fori_loop(0, NP, phase, 0)

        out = pl.pallas_call(
            kernel,
            in_specs=[pl.BlockSpec(memory_space=pl.ANY)] * 3,
            out_specs=pl.BlockSpec(memory_space=pl.ANY),
            out_shape=jax.ShapeDtypeStruct(x5.shape, x.dtype),
            scratch_shapes=[
                pltpu.VMEM(((RING + 1) * S, 2, SH, RS, W), x.dtype),
                pltpu.VMEM((2, 8, C // 8), g.dtype),
                pltpu.VMEM((16, C // 8), jnp.float32),
                pltpu.SMEM((16, C // 8), jnp.float32),
                pltpu.SemaphoreType.DMA((1,)),
            ],
            compiler_params=pltpu.CompilerParams(
                vmem_limit_bytes=(RING + 1) * 8 * 1024 * 1024 + 8 * 1024 * 1024,
                disable_bounds_checks=nobounds),
        )(x5, g2, b2)
        return out.reshape(x.shape)
    return fn


pallas_standalone__groupnorm__prompt_kernel = _make_kernel()
```

```python
import jax
import jax.numpy as jnp
from jax import lax
import jax.experimental.pallas as pl
import jax.experimental.pallas.tpu as pltpu

EPS = 1e-5
NUM_GROUPS = 32

D = 16
DH = 8
RW_LEAD = 7
TJ = 4
TW = 2
RCW = 256
WCW = 1024
AW = 256
HK = 2


def _shr(v, n):
    return v >> n if isinstance(v, int) else lax.shift_right_logical(v, jnp.int32(n))


def _and(v, m):
    return v & m if isinstance(v, int) else lax.bitwise_and(v, jnp.int32(m))


def _sel(p, vals):
    r = jnp.int32(vals[0])
    for i in range(1, len(vals)):
        r = jnp.where(p == i, jnp.int32(vals[i]), r)
    return r


@jax.jit
def pallas_standalone__groupnorm__prompt_kernel(
    x: jax.Array,
    g: jax.Array,
    b: jax.Array,
):
    B, C, H, W = x.shape
    assert (B, C, H, W) == (2, 1024, 32, 2048)
    G = NUM_GROUPS
    cpg = C // G
    RS = 8
    SPC = H // RS
    CPS = 8
    SH = CPS * SPC // 2
    NSTR = B * C // CPS
    S = 8
    SHIFT = 2
    V = NSTR // S - 1
    RING = 11
    RJ = W // RCW
    SPW = SH * RJ
    LSPW = SPW.bit_length() - 1
    LRJ = RJ.bit_length() - 1
    NSL = 3 * cpg * HK
    WJ = W // WCW
    TCW = W // TJ
    NHS = 2 * DH
    n_el = cpg * H * W
    KR0 = (0, 11, 21)
    NWR = (11, 10, 10)
    GA = (0, 22, 42)
    LEAD = (4, 2, 2)
    NM = (18, 18, 20)
    KA = (0, 10, 20)
    NKW = (10, 10, 11)
    NP = 3
    assert SPW % D == 0 and D % NHS == 0 and RW_LEAD < D
    assert all(SPW + l * NSL <= n * SPW - D for l, n in zip(LEAD, NWR)) and 2 * NSL >= SPW

    x5 = x.reshape(NSTR, 2, SH, RS, W)
    g2 = g.reshape(8, C // 8)
    b2 = b.reshape(8, C // 8)

    def body(x_hbm, g_hbm, b_hbm, o_hbm, buf, gb_bf, gb_f32, gb_s, lsem, hsem, wsem, tsem, vsem, psem):
        def pos_of(k):
            if isinstance(k, int):
                return k % RING
            return k - jnp.where(k >= 2 * RING, 2 * RING, jnp.where(k >= RING, RING, 0))

        def start(copies, priority):
            for c in copies:
                c.start(priority=priority)

        def wait(copies):
            for c in copies:
                c.wait()

        def rd(n0, v0, ns, u, sem):
            sl = _shr(u, LRJ)
            c0 = _and(u, RJ - 1) * RCW
            cs = pl.ds(c0 if isinstance(c0, int) else pl.multiple_of(c0, RCW), RCW)
            return pltpu.make_async_copy(
                x_hbm.at[pl.ds(n0, ns), :, sl, :, cs], buf.at[pl.ds(v0, ns), :, sl, :, cs], sem)

        def low(kr0, j):
            k = kr0 + _shr(j, LSPW)
            return [rd(k * S + SHIFT, pos_of(k) * S, S - 1, _and(j, SPW - 1), lsem.at[_and(j, D - 1)])]

        def high(kr0, j):
            k = kr0 + _shr(j, LSPW)
            return [rd(k * S + SHIFT + S - 1, pos_of(k) * S + S - 1, 1, _and(j, SPW - 1),
                       hsem.at[_and(j, NHS - 1)])]

        def low_v(j):
            sem = lsem.at[_and(j, D - 1)]
            return [rd(V * S + SHIFT, RING * S, S - SHIFT, j, sem),
                    rd(0, RING * S + S - SHIFT, SHIFT - 1, j, sem)]

        def high_v(j):
            return [rd(SHIFT - 1, RING * S + S - 1, 1, j, hsem.at[_and(j, NHS - 1)])]

        def wr(n0, v0, ns, half, sl, cs, sem):
            return pltpu.make_async_copy(buf.at[pl.ds(v0, ns), half, sl, :, cs],
                                         o_hbm.at[pl.ds(n0, ns), half, sl, :, cs], sem)

        def tail(k, t):
            pos = pos_of(k)
            return wr(k * S + SHIFT, pos * S, S, 1, SH - 1, pl.ds(t * TCW, TCW), tsem.at[TJ * pos + t])

        def issue_chunk(cid):
            k = _shr(cid, 1)
            half = _and(cid, 1)
            pos = pos_of(k)

            def slab(sl, c):
                for jj in range(WJ):
                    wr(k * S + SHIFT, pos * S, S, half, sl, pl.ds(jj * WCW, WCW),
                       wsem.at[2 * pos + half]).start()
                return c
            lax.fori_loop(0, SH - half, slab, 0)

            @pl.when(half == 1)
            def _():
                for t in range(TJ):
                    tail(k, t).start()

        def wait_head(k):
            pos = pos_of(k)
            wr(k * S + SHIFT, pos * S, S, 0, pl.ds(0, SH), pl.ds(0, W), wsem.at[2 * pos]).wait()
            wr(k * S + SHIFT, pos * S, S, 1, pl.ds(0, SH - 1), pl.ds(0, W), wsem.at[2 * pos + 1]).wait()

        parts_v = ((V * S + SHIFT, RING * S, S - SHIFT), (0, RING * S + S - SHIFT, SHIFT))

        def tree(parts):
            while len(parts) > 1:
                parts = [parts[i] + parts[i + 1] for i in range(0, len(parts), 2)]
            return parts[0]

        def compute_group(gi, hook, cu):
            def vstream(s):
                n = _and(gi * 4 + s - SHIFT, NSTR - 1)
                k = _shr(n, 3)
                return jnp.where(k == V, RING, pos_of(k)) * S + _and(n, S - 1)
            nit = cpg // cu

            def refs(it):
                if cu == CPS:
                    base = buf.at[vstream(it)]
                    return [base.at[c // 4, pl.ds((c % 4) * SPC, SPC)] for c in range(cu)]
                assert cu == 1
                return [buf.at[vstream(_shr(it, 3)), _and(_shr(it, 2), 1), pl.ds(_and(it, 3) * SPC, SPC)]]

            def red(r, f, hk):
                outs = []
                for k in range(SPC):
                    if k % (SPC // HK) == 0:
                        hook(hk * HK + k // (SPC // HK))
                    v = f(r[k].astype(jnp.float32))
                    outs.append(tree([v[:, j * AW:(j + 1) * AW] for j in range(W // AW)]))
                return tree(outs)

            def p1(it, acc):
                for c, r in enumerate(refs(it)):
                    acc = acc + red(r, lambda v: v, it * cu + c)
                return acc
            acc = lax.fori_loop(0, nit, p1, jnp.zeros((RS, AW), jnp.float32))
            mu = jnp.sum(acc, keepdims=True) * (1.0 / n_el)

            def sq(v):
                d = v - mu
                return d * d

            def p2(it, acc):
                for c, r in enumerate(refs(it)):
                    acc = acc + red(r, sq, cpg + it * cu + c)
                return acc
            acc = lax.fori_loop(0, nit, p2, jnp.zeros((RS, AW), jnp.float32))
            var = jnp.sum(acc, keepdims=True) * (1.0 / n_el)
            rstd = lax.rsqrt(var + EPS)
            cb = _and(gi, G - 1) * cpg
            crow = _shr(cb, 7)
            ccol = _and(cb, 127)

            def p3(it, carry):
                for c, r in enumerate(refs(it)):
                    ch = ccol + it * cu + c
                    a = rstd * gb_s[crow, ch]
                    sh = gb_s[8 + crow, ch]
                    for hh in range(HK):
                        hook((2 * cpg + it * cu + c) * HK + hh)
                        rr = r.at[pl.ds(hh * (SPC // HK), SPC // HK)]
                        rr[...] = ((rr[...].astype(jnp.float32) - mu) * a + sh).astype(buf.dtype)
                return carry
            lax.fori_loop(0, nit, p3, 0)

        for j in range(DH):
            start(high_v(j), 0)
        for j in range(D):
            start(low_v(j), 1)
        cp_g = pltpu.make_async_copy(g_hbm, gb_bf.at[0], psem.at[0])
        cp_b = pltpu.make_async_copy(b_hbm, gb_bf.at[1], psem.at[1])
        cp_g.start()
        cp_b.start()

        def pace_v(j, c):
            wait(low_v(j))
            wait(high_v(j))
            start(high_v(j + DH), 0)
            start(low_v(j + D), 1)
            return c
        lax.fori_loop(0, 16, pace_v, 0)
        cp_g.wait()
        cp_b.wait()
        gb_f32[0:8, :] = gb_bf[0].astype(jnp.float32)
        gb_f32[8:16, :] = gb_bf[1].astype(jnp.float32)
        cp_s = pltpu.make_async_copy(gb_f32, gb_s, psem.at[2])
        cp_s.start()
        lax.fori_loop(16, SPW - D, pace_v, 0)
        cp_s.wait()
        for j in range(SPW - D, SPW):
            wait(low_v(j))
            wait(high_v(j))
            start(high_v(j + DH) if j + DH < SPW else high(0, j + DH - SPW), 0)
            start(low(0, j + D - SPW), 1)

        def phase(p, carry):
            kr0 = _sel(p, KR0)
            nsteps = _sel(p, NWR) * SPW
            ga = _sel(p, GA)
            lead = _sel(p, LEAD)
            ka = _sel(p, KA)

            def pace(j):
                wait(low(kr0, j))
                wait(high(kr0, j))
                start(high(kr0, j + DH), 0)
                start(low(kr0, j + D), 1)

            def pace_loop(lo, hi):
                def step(j, c):
                    pace(j)
                    return c
                lax.fori_loop(lo, hi, step, 0)

            pace_loop(0, SPW)

            def lead_group(q, c):
                compute_group(ga + q, lambda k: pace(SPW + q * NSL + k), 1)
                return c
            lax.fori_loop(0, lead, lead_group, 0)
            pace_loop(SPW + lead * NSL, nsteps - D)
            for t in range(D):
                j = nsteps - D + t
                wait(low(kr0, j))
                wait(high(kr0, j))
                if t + DH < D:
                    start(high(kr0, j + DH), 0)
                if t == D - 1 - RW_LEAD:
                    issue_chunk(2 * ka)
            issue_chunk(2 * ka + 1)

            def write_group(m, c):
                compute_group(ga + lead + m, lambda k: None, CPS)
                issue_chunk(2 * ka + 2 + m)
                return c
            lax.fori_loop(0, _sel(p, NM), write_group, 0)

            @pl.when(p == NP - 1)
            def _():
                for half in range(2):
                    def slab_v(sl, c):
                        for jj in range(WJ):
                            for i, (n0, v0, ns) in enumerate(parts_v):
                                wr(n0, v0, ns, half, sl, pl.ds(jj * WCW, WCW), vsem.at[i]).start()
                        return c
                    lax.fori_loop(0, SH, slab_v, 0)

            k_last = ka + _sel(p, NKW) - 1

            def wait_window(k, c):
                wait_head(k)
                for t in range(TJ):
                    tail(k, t).wait()
                return c
            lax.fori_loop(ka, k_last, wait_window, 0)
            wait_head(k_last)
            for t in range(TW):
                tail(k_last, t).wait()

            @pl.when(p < NP - 1)
            def _():
                kr_next = kr0 + _sel(p, NWR)
                for j in range(DH):
                    start(high(kr_next, j), 0)
                for j in range(D):
                    start(low(kr_next, j), 1)
            for t in range(TW, TJ):
                tail(k_last, t).wait()
            return carry
        lax.fori_loop(0, NP, phase, 0)
        for i, (n0, v0, ns) in enumerate(parts_v):
            pltpu.make_async_copy(buf.at[pl.ds(v0, ns)], o_hbm.at[pl.ds(n0, ns)], vsem.at[i]).wait()

    def kernel(*refs):
        pl.run_scoped(
            lambda *sems: body(*refs, *sems),
            pltpu.SemaphoreType.DMA((D,)),
            pltpu.SemaphoreType.DMA((NHS,)),
            pltpu.SemaphoreType.DMA((2 * RING,)),
            pltpu.SemaphoreType.DMA((TJ * RING,)),
            pltpu.SemaphoreType.DMA((2,)),
            pltpu.SemaphoreType.DMA((3,)))

    out = pl.pallas_call(
        kernel,
        in_specs=[pl.BlockSpec(memory_space=pl.ANY)] * 3,
        out_specs=pl.BlockSpec(memory_space=pl.ANY),
        out_shape=jax.ShapeDtypeStruct(x5.shape, x.dtype),
        scratch_shapes=[
            pltpu.VMEM(((RING + 1) * S, 2, SH, RS, W), x.dtype),
            pltpu.VMEM((2, 8, C // 8), g.dtype),
            pltpu.VMEM((16, C // 8), jnp.float32),
            pltpu.SMEM((16, C // 8), jnp.float32),
        ],
        compiler_params=pltpu.CompilerParams(
            vmem_limit_bytes=(RING + 2) * 8 * 1024 * 1024,
            disable_bounds_checks=True),
    )(x5, g2, b2)
    return out.reshape(x.shape)
```

```python
import jax
import jax.numpy as jnp
from jax import lax
import jax.experimental.pallas as pl
import jax.experimental.pallas.tpu as pltpu

EPS = 1e-5
NUM_GROUPS = 32

D = 16
DH = 8
RW_LEAD = 7
TJ = 4
TW = 2
RCW = 256
RPC = 128
WPC = (640, 640, 768)
AW = 256
HK = 2


def _shr(v, n):
    return v >> n if isinstance(v, int) else lax.shift_right_logical(v, jnp.int32(n))


def _and(v, m):
    return v & m if isinstance(v, int) else lax.bitwise_and(v, jnp.int32(m))


def _sel(p, vals):
    r = jnp.int32(vals[0])
    for i in range(1, len(vals)):
        r = jnp.where(p == i, jnp.int32(vals[i]), r)
    return r


@jax.jit
def pallas_standalone__groupnorm__prompt_kernel(
    x: jax.Array,
    g: jax.Array,
    b: jax.Array,
):
    B, C, H, W = x.shape
    assert (B, C, H, W) == (2, 1024, 32, 2048)
    G = NUM_GROUPS
    cpg = C // G
    RS = 8
    SPC = H // RS
    CPS = 8
    SH = CPS * SPC // 2
    NSTR = B * C // CPS
    S = 8
    SHIFT = 2
    V = NSTR // S - 1
    RING = 11
    RJ = W // RCW
    SPW = SH * RJ
    LSPW = SPW.bit_length() - 1
    LRJ = RJ.bit_length() - 1
    NSL = 3 * cpg * HK
    assert sum(WPC) == W
    wcols = [pl.ds(sum(WPC[:i]), WPC[i]) for i in range(len(WPC))]
    TCW = W // TJ
    NHS = 2 * DH
    n_el = cpg * H * W
    KR0 = (0, 11, 21)
    NWR = (11, 10, 10)
    GA = (0, 22, 42)
    LEAD = (4, 2, 2)
    NM = (18, 18, 20)
    KA = (0, 10, 20)
    NKW = (10, 10, 11)
    NP = 3
    assert SPW % D == 0 and D % NHS == 0 and RW_LEAD < D
    assert all(SPW + l * NSL <= n * SPW - D for l, n in zip(LEAD, NWR)) and 2 * NSL >= SPW

    x5 = x.reshape(NSTR, 2, SH, RS, W)
    g2 = g.reshape(8, C // 8)
    b2 = b.reshape(8, C // 8)

    def body(x_hbm, g_hbm, b_hbm, o_hbm, buf, gb_bf, gb_f32, gb_s, lsem, hsem, wsem, tsem, vsem, psem):
        def pos_of(k):
            if isinstance(k, int):
                return k % RING
            return k - jnp.where(k >= 2 * RING, 2 * RING, jnp.where(k >= RING, RING, 0))

        def start(copies, priority):
            for c in copies:
                c.start(priority=priority)

        def wait(copies):
            for c in copies:
                c.wait()

        def rd(parts, u, sem):
            sl = _shr(u, LRJ)
            c0 = _and(u, RJ - 1) * RCW
            cs = pl.ds(c0 if isinstance(c0, int) else pl.multiple_of(c0, RCW), RCW)
            views = [(x_hbm.at[pl.ds(n0, ns), :, sl, :, cs], buf.at[pl.ds(v0, ns), :, sl, :, cs])
                     for n0, v0, ns in parts]
            return [pltpu.make_async_copy(src.at[:, :, :, pl.ds(c, RPC)], dst.at[:, :, :, pl.ds(c, RPC)], sem)
                    for c in range(0, RCW, RPC) for src, dst in views]

        def low(kr0, j):
            k = kr0 + _shr(j, LSPW)
            return rd([(k * S + SHIFT, pos_of(k) * S, S - 1)], _and(j, SPW - 1), lsem.at[_and(j, D - 1)])

        def high(kr0, j):
            k = kr0 + _shr(j, LSPW)
            return rd([(k * S + SHIFT + S - 1, pos_of(k) * S + S - 1, 1)], _and(j, SPW - 1),
                      hsem.at[_and(j, NHS - 1)])

        def low_v(j):
            return rd([(V * S + SHIFT, RING * S, S - SHIFT), (0, RING * S + S - SHIFT, SHIFT - 1)], j,
                      lsem.at[_and(j, D - 1)])

        def high_v(j):
            return rd([(SHIFT - 1, RING * S + S - 1, 1)], j, hsem.at[_and(j, NHS - 1)])

        def wr(n0, v0, ns, half, sl, cs, sem):
            return pltpu.make_async_copy(buf.at[pl.ds(v0, ns), half, sl, :, cs],
                                         o_hbm.at[pl.ds(n0, ns), half, sl, :, cs], sem)

        def tail(k, t):
            pos = pos_of(k)
            return wr(k * S + SHIFT, pos * S, S, 1, SH - 1, pl.ds(t * TCW, TCW), tsem.at[TJ * pos + t])

        def issue_chunk(cid):
            k = _shr(cid, 1)
            half = _and(cid, 1)
            pos = pos_of(k)

            def slab(sl, c):
                for cs in wcols:
                    wr(k * S + SHIFT, pos * S, S, half, sl, cs, wsem.at[2 * pos + half]).start()
                return c
            lax.fori_loop(0, SH - half, slab, 0)

            @pl.when(half == 1)
            def _():
                for t in range(TJ):
                    tail(k, t).start()

        def wait_head(k):
            pos = pos_of(k)
            wr(k * S + SHIFT, pos * S, S, 0, pl.ds(0, SH), pl.ds(0, W), wsem.at[2 * pos]).wait()
            wr(k * S + SHIFT, pos * S, S, 1, pl.ds(0, SH - 1), pl.ds(0, W), wsem.at[2 * pos + 1]).wait()

        parts_v = ((V * S + SHIFT, RING * S, S - SHIFT), (0, RING * S + S - SHIFT, SHIFT))

        def tree(parts):
            while len(parts) > 1:
                parts = [parts[i] + parts[i + 1] for i in range(0, len(parts), 2)]
            return parts[0]

        def compute_group(gi, hook, cu):
            def vstream(s):
                n = _and(gi * 4 + s - SHIFT, NSTR - 1)
                k = _shr(n, 3)
                return jnp.where(k == V, RING, pos_of(k)) * S + _and(n, S - 1)
            nit = cpg // cu

            def refs(it):
                if cu == CPS:
                    base = buf.at[vstream(it)]
                    return [base.at[c // 4, pl.ds((c % 4) * SPC, SPC)] for c in range(cu)]
                assert cu == 1
                return [buf.at[vstream(_shr(it, 3)), _and(_shr(it, 2), 1), pl.ds(_and(it, 3) * SPC, SPC)]]

            def red(r, f, hk):
                outs = []
                for k in range(SPC):
                    if k % (SPC // HK) == 0:
                        hook(hk * HK + k // (SPC // HK))
                    v = f(r[k].astype(jnp.float32))
                    outs.append(tree([v[:, j * AW:(j + 1) * AW] for j in range(W // AW)]))
                return tree(outs)

            def p1(it, acc):
                for c, r in enumerate(refs(it)):
                    acc = acc + red(r, lambda v: v, it * cu + c)
                return acc
            acc = lax.fori_loop(0, nit, p1, jnp.zeros((RS, AW), jnp.float32))
            mu = jnp.sum(acc, keepdims=True) * (1.0 / n_el)

            def sq(v):
                d = v - mu
                return d * d

            def p2(it, acc):
                for c, r in enumerate(refs(it)):
                    acc = acc + red(r, sq, cpg + it * cu + c)
                return acc
            acc = lax.fori_loop(0, nit, p2, jnp.zeros((RS, AW), jnp.float32))
            var = jnp.sum(acc, keepdims=True) * (1.0 / n_el)
            rstd = lax.rsqrt(var + EPS)
            cb = _and(gi, G - 1) * cpg
            crow = _shr(cb, 7)
            ccol = _and(cb, 127)

            def p3(it, carry):
                for c, r in enumerate(refs(it)):
                    ch = ccol + it * cu + c
                    a = rstd * gb_s[crow, ch]
                    sh = gb_s[8 + crow, ch]
                    for hh in range(HK):
                        hook((2 * cpg + it * cu + c) * HK + hh)
                        rr = r.at[pl.ds(hh * (SPC // HK), SPC // HK)]
                        rr[...] = ((rr[...].astype(jnp.float32) - mu) * a + sh).astype(buf.dtype)
                return carry
            lax.fori_loop(0, nit, p3, 0)

        for j in range(DH):
            start(high_v(j), 0)
        for j in range(D):
            start(low_v(j), 1)
        cp_g = pltpu.make_async_copy(g_hbm, gb_bf.at[0], psem.at[0])
        cp_b = pltpu.make_async_copy(b_hbm, gb_bf.at[1], psem.at[1])
        cp_g.start()
        cp_b.start()

        def pace_v(j, c):
            wait(low_v(j))
            wait(high_v(j))
            start(high_v(j + DH), 0)
            start(low_v(j + D), 1)
            return c
        lax.fori_loop(0, 16, pace_v, 0)
        cp_g.wait()
        cp_b.wait()
        gb_f32[0:8, :] = gb_bf[0].astype(jnp.float32)
        gb_f32[8:16, :] = gb_bf[1].astype(jnp.float32)
        cp_s = pltpu.make_async_copy(gb_f32, gb_s, psem.at[2])
        cp_s.start()
        lax.fori_loop(16, SPW - D, pace_v, 0)
        cp_s.wait()
        for j in range(SPW - D, SPW):
            wait(low_v(j))
            wait(high_v(j))
            start(high_v(j + DH) if j + DH < SPW else high(0, j + DH - SPW), 0)
            start(low(0, j + D - SPW), 1)

        def phase(p, carry):
            kr0 = _sel(p, KR0)
            nsteps = _sel(p, NWR) * SPW
            ga = _sel(p, GA)
            lead = _sel(p, LEAD)
            ka = _sel(p, KA)

            def pace(j):
                wait(low(kr0, j))
                wait(high(kr0, j))
                start(high(kr0, j + DH), 0)
                start(low(kr0, j + D), 1)

            def pace_loop(lo, hi):
                def step(j, c):
                    pace(j)
                    return c
                lax.fori_loop(lo, hi, step, 0)

            pace_loop(0, SPW)

            def lead_group(q, c):
                compute_group(ga + q, lambda k: pace(SPW + q * NSL + k), 1)
                return c
            lax.fori_loop(0, lead, lead_group, 0)
            pace_loop(SPW + lead * NSL, nsteps - D)
            for t in range(D):
                j = nsteps - D + t
                wait(low(kr0, j))
                wait(high(kr0, j))
                if t + DH < D:
                    start(high(kr0, j + DH), 0)
                if t == D - 1 - RW_LEAD:
                    issue_chunk(2 * ka)
            issue_chunk(2 * ka + 1)

            def write_group(m, c):
                compute_group(ga + lead + m, lambda k: None, CPS)
                issue_chunk(2 * ka + 2 + m)
                return c
            lax.fori_loop(0, _sel(p, NM), write_group, 0)

            @pl.when(p == NP - 1)
            def _():
                for half in range(2):
                    def slab_v(sl, c):
                        for cs in wcols:
                            for i, (n0, v0, ns) in enumerate(parts_v):
                                wr(n0, v0, ns, half, sl, cs, vsem.at[i]).start()
                        return c
                    lax.fori_loop(0, SH, slab_v, 0)

            k_last = ka + _sel(p, NKW) - 1

            def wait_window(k, c):
                wait_head(k)
                for t in range(TJ):
                    tail(k, t).wait()
                return c
            lax.fori_loop(ka, k_last, wait_window, 0)
            wait_head(k_last)
            for t in range(TW):
                tail(k_last, t).wait()

            @pl.when(p < NP - 1)
            def _():
                kr_next = kr0 + _sel(p, NWR)
                for j in range(DH):
                    start(high(kr_next, j), 0)
                for j in range(D):
                    start(low(kr_next, j), 1)
            for t in range(TW, TJ):
                tail(k_last, t).wait()
            return carry
        lax.fori_loop(0, NP, phase, 0)
        for i, (n0, v0, ns) in enumerate(parts_v):
            pltpu.make_async_copy(buf.at[pl.ds(v0, ns)], o_hbm.at[pl.ds(n0, ns)], vsem.at[i]).wait()

    def kernel(*refs):
        pl.run_scoped(
            lambda *sems: body(*refs, *sems),
            pltpu.SemaphoreType.DMA((D,)),
            pltpu.SemaphoreType.DMA((NHS,)),
            pltpu.SemaphoreType.DMA((2 * RING,)),
            pltpu.SemaphoreType.DMA((TJ * RING,)),
            pltpu.SemaphoreType.DMA((2,)),
            pltpu.SemaphoreType.DMA((3,)))

    out = pl.pallas_call(
        kernel,
        in_specs=[pl.BlockSpec(memory_space=pl.ANY)] * 3,
        out_specs=pl.BlockSpec(memory_space=pl.ANY),
        out_shape=jax.ShapeDtypeStruct(x5.shape, x.dtype),
        scratch_shapes=[
            pltpu.VMEM(((RING + 1) * S, 2, SH, RS, W), x.dtype),
            pltpu.VMEM((2, 8, C // 8), g.dtype),
            pltpu.VMEM((16, C // 8), jnp.float32),
            pltpu.SMEM((16, C // 8), jnp.float32),
        ],
        compiler_params=pltpu.CompilerParams(
            vmem_limit_bytes=(RING + 2) * 8 * 1024 * 1024,
            disable_bounds_checks=True),
    )(x5, g2, b2)
    return out.reshape(x.shape)
```

```python
import jax
import jax.numpy as jnp
from jax import lax
import jax.experimental.pallas as pl
import jax.experimental.pallas.tpu as pltpu

EPS = 1e-5
NUM_GROUPS = 32

D = 16
DH = 10
RW_LEAD = 7
TJ = 4
TW = 2
RCW = 256
RPC = 128
WPC = (640, 640, 768)
AW = 256
HK = 2


def _shr(v, n):
    return v >> n if isinstance(v, int) else lax.shift_right_logical(v, jnp.int32(n))


def _and(v, m):
    return v & m if isinstance(v, int) else lax.bitwise_and(v, jnp.int32(m))


def _sel(p, vals):
    r = jnp.int32(vals[0])
    for i in range(1, len(vals)):
        r = jnp.where(p == i, jnp.int32(vals[i]), r)
    return r


@jax.jit
def pallas_standalone__groupnorm__prompt_kernel(
    x: jax.Array,
    g: jax.Array,
    b: jax.Array,
):
    B, C, H, W = x.shape
    assert (B, C, H, W) == (2, 1024, 32, 2048)
    G = NUM_GROUPS
    cpg = C // G
    RS = 8
    SPC = H // RS
    CPS = 8
    SH = CPS * SPC // 2
    NSTR = B * C // CPS
    S = 8
    SHIFT = 2
    V = NSTR // S - 1
    RING = 11
    RJ = W // RCW
    SPW = SH * RJ
    LSPW = SPW.bit_length() - 1
    LRJ = RJ.bit_length() - 1
    NSL = 3 * cpg * HK
    assert sum(WPC) == W
    wcols = [pl.ds(sum(WPC[:i]), WPC[i]) for i in range(len(WPC))]
    TCW = W // TJ
    n_el = cpg * H * W
    KR0 = (0, 11, 21)
    NWR = (11, 10, 10)
    GA = (0, 22, 42)
    LEAD = (4, 2, 2)
    NM = (18, 18, 20)
    KA = (0, 10, 20)
    NKW = (10, 10, 11)
    NP = 3
    assert SPW % D == 0 and DH <= D and RW_LEAD < D
    assert all(SPW + l * NSL <= n * SPW - D for l, n in zip(LEAD, NWR)) and 2 * NSL >= SPW

    x5 = x.reshape(NSTR, 2, SH, RS, W)
    g2 = g.reshape(8, C // 8)
    b2 = b.reshape(8, C // 8)

    def body(x_hbm, g_hbm, b_hbm, o_hbm, buf, gb_bf, gb_f32, gb_s, lsem, hsem, wsem, tsem, vsem, psem):
        def pos_of(k):
            if isinstance(k, int):
                return k % RING
            return k - jnp.where(k >= 2 * RING, 2 * RING, jnp.where(k >= RING, RING, 0))

        def start(copies, priority):
            for c in copies:
                c.start(priority=priority)

        def wait(copies):
            for c in copies:
                c.wait()

        def rd(n0, v0, ns, u, sem):
            sl = _shr(u, LRJ)
            c0 = _and(u, RJ - 1) * RCW
            cs = pl.ds(c0 if isinstance(c0, int) else pl.multiple_of(c0, RCW), RCW)
            src = x_hbm.at[pl.ds(n0, ns), :, sl, :, cs]
            dst = buf.at[pl.ds(v0, ns), :, sl, :, cs]
            return [pltpu.make_async_copy(src.at[:, :, :, pl.ds(c, RPC)], dst.at[:, :, :, pl.ds(c, RPC)], sem)
                    for c in range(0, RCW, RPC)]

        def low(kr0, j):
            k = kr0 + _shr(j, LSPW)
            return rd(k * S + SHIFT, pos_of(k) * S, S - 1, _and(j, SPW - 1), lsem.at[_and(j, D - 1)])

        def high(kr0, j):
            k = kr0 + _shr(j, LSPW)
            return rd(k * S + SHIFT + S - 1, pos_of(k) * S + S - 1, 1, _and(j, SPW - 1),
                      hsem.at[_and(j, D - 1)])

        parts_v = ((V * S + SHIFT, RING * S, S - SHIFT), (0, RING * S + S - SHIFT, SHIFT))

        def low_v(j):
            return rd(*parts_v[0], j, lsem.at[_and(j, D - 1)])

        def high_v(j):
            return rd(*parts_v[1], j, hsem.at[_and(j, D - 1)])

        def wr(n0, v0, ns, half, sl, cs, sem):
            return pltpu.make_async_copy(buf.at[pl.ds(v0, ns), half, sl, :, cs],
                                         o_hbm.at[pl.ds(n0, ns), half, sl, :, cs], sem)

        def tail(k, t):
            pos = pos_of(k)
            return wr(k * S + SHIFT, pos * S, S, 1, SH - 1, pl.ds(t * TCW, TCW), tsem.at[TJ * pos + t])

        def issue_chunk(cid):
            k = _shr(cid, 1)
            half = _and(cid, 1)
            pos = pos_of(k)

            def slab(sl, c):
                for cs in wcols:
                    wr(k * S + SHIFT, pos * S, S, half, sl, cs, wsem.at[2 * pos + half]).start()
                return c
            lax.fori_loop(0, SH - half, slab, 0)

            @pl.when(half == 1)
            def _():
                for t in range(TJ):
                    tail(k, t).start()

        def wait_head(k):
            pos = pos_of(k)
            wr(k * S + SHIFT, pos * S, S, 0, pl.ds(0, SH), pl.ds(0, W), wsem.at[2 * pos]).wait()
            wr(k * S + SHIFT, pos * S, S, 1, pl.ds(0, SH - 1), pl.ds(0, W), wsem.at[2 * pos + 1]).wait()

        def tree(parts):
            while len(parts) > 1:
                parts = [parts[i] + parts[i + 1] for i in range(0, len(parts), 2)]
            return parts[0]

        def compute_group(gi, hook, cu):
            def vstream(s):
                n = _and(gi * 4 + s - SHIFT, NSTR - 1)
                k = _shr(n, 3)
                return jnp.where(k == V, RING, pos_of(k)) * S + _and(n, S - 1)
            nit = cpg // cu

            def refs(it):
                if cu == CPS:
                    base = buf.at[vstream(it)]
                    return [base.at[c // 4, pl.ds((c % 4) * SPC, SPC)] for c in range(cu)]
                assert cu == 1
                return [buf.at[vstream(_shr(it, 3)), _and(_shr(it, 2), 1), pl.ds(_and(it, 3) * SPC, SPC)]]

            def red(r, f, hk):
                outs = []
                for k in range(SPC):
                    if k % (SPC // HK) == 0:
                        hook(hk * HK + k // (SPC // HK))
                    v = f(r[k].astype(jnp.float32))
                    outs.append(tree([v[:, j * AW:(j + 1) * AW] for j in range(W // AW)]))
                return tree(outs)

            def p1(it, acc):
                for c, r in enumerate(refs(it)):
                    acc = acc + red(r, lambda v: v, it * cu + c)
                return acc
            acc = lax.fori_loop(0, nit, p1, jnp.zeros((RS, AW), jnp.float32))
            mu = jnp.sum(acc, keepdims=True) * (1.0 / n_el)

            def sq(v):
                d = v - mu
                return d * d

            def p2(it, acc):
                for c, r in enumerate(refs(it)):
                    acc = acc + red(r, sq, cpg + it * cu + c)
                return acc
            acc = lax.fori_loop(0, nit, p2, jnp.zeros((RS, AW), jnp.float32))
            var = jnp.sum(acc, keepdims=True) * (1.0 / n_el)
            rstd = lax.rsqrt(var + EPS)
            cb = _and(gi, G - 1) * cpg
            crow = _shr(cb, 7)
            ccol = _and(cb, 127)

            def p3(it, carry):
                for c, r in enumerate(refs(it)):
                    ch = ccol + it * cu + c
                    a = rstd * gb_s[crow, ch]
                    sh = gb_s[8 + crow, ch]
                    for hh in range(HK):
                        hook((2 * cpg + it * cu + c) * HK + hh)
                        rr = r.at[pl.ds(hh * (SPC // HK), SPC // HK)]
                        rr[...] = ((rr[...].astype(jnp.float32) - mu) * a + sh).astype(buf.dtype)
                return carry
            lax.fori_loop(0, nit, p3, 0)

        for j in range(DH):
            start(high_v(j), 0)
        for j in range(D):
            start(low_v(j), 1)
        cp_g = pltpu.make_async_copy(g_hbm, gb_bf.at[0], psem.at[0])
        cp_b = pltpu.make_async_copy(b_hbm, gb_bf.at[1], psem.at[1])
        cp_g.start()
        cp_b.start()

        def pace_v(j, c):
            wait(low_v(j))
            wait(high_v(j))
            start(high_v(j + DH), 0)
            start(low_v(j + D), 1)
            return c
        lax.fori_loop(0, 16, pace_v, 0)
        cp_g.wait()
        cp_b.wait()
        gb_f32[0:8, :] = gb_bf[0].astype(jnp.float32)
        gb_f32[8:16, :] = gb_bf[1].astype(jnp.float32)
        cp_s = pltpu.make_async_copy(gb_f32, gb_s, psem.at[2])
        cp_s.start()
        lax.fori_loop(16, SPW - D, pace_v, 0)
        cp_s.wait()
        for j in range(SPW - D, SPW):
            wait(low_v(j))
            wait(high_v(j))
            start(high_v(j + DH) if j + DH < SPW else high(0, j + DH - SPW), 0)
            start(low(0, j + D - SPW), 1)

        def phase(p, carry):
            kr0 = _sel(p, KR0)
            nsteps = _sel(p, NWR) * SPW
            ga = _sel(p, GA)
            lead = _sel(p, LEAD)
            ka = _sel(p, KA)

            def pace(j):
                wait(low(kr0, j))
                wait(high(kr0, j))
                start(high(kr0, j + DH), 0)
                start(low(kr0, j + D), 1)

            def pace_loop(lo, hi):
                def step(j, c):
                    pace(j)
                    return c
                lax.fori_loop(lo, hi, step, 0)

            pace_loop(0, SPW)

            def lead_group(q, c):
                compute_group(ga + q, lambda k: pace(SPW + q * NSL + k), 1)
                return c
            lax.fori_loop(0, lead, lead_group, 0)
            pace_loop(SPW + lead * NSL, nsteps - D)
            for t in range(D):
                j = nsteps - D + t
                wait(low(kr0, j))
                wait(high(kr0, j))
                if t + DH < D:
                    start(high(kr0, j + DH), 0)
                if t == D - 1 - RW_LEAD:
                    issue_chunk(2 * ka)
            issue_chunk(2 * ka + 1)

            def write_group(m, c):
                compute_group(ga + lead + m, lambda k: None, CPS)
                issue_chunk(2 * ka + 2 + m)
                return c
            lax.fori_loop(0, _sel(p, NM), write_group, 0)

            @pl.when(p == NP - 1)
            def _():
                for half in range(2):
                    def slab_v(sl, c):
                        for cs in wcols:
                            for i, (n0, v0, ns) in enumerate(parts_v):
                                wr(n0, v0, ns, half, sl, cs, vsem.at[i]).start()
                        return c
                    lax.fori_loop(0, SH, slab_v, 0)

            k_last = ka + _sel(p, NKW) - 1

            def wait_window(k, c):
                wait_head(k)
                for t in range(TJ):
                    tail(k, t).wait()
                return c
            lax.fori_loop(ka, k_last, wait_window, 0)
            wait_head(k_last)
            for t in range(TW):
                tail(k_last, t).wait()

            @pl.when(p < NP - 1)
            def _():
                kr_next = kr0 + _sel(p, NWR)
                for j in range(DH):
                    start(high(kr_next, j), 0)
                for j in range(D):
                    start(low(kr_next, j), 1)
            for t in range(TW, TJ):
                tail(k_last, t).wait()
            return carry
        lax.fori_loop(0, NP, phase, 0)
        for i, (n0, v0, ns) in enumerate(parts_v):
            pltpu.make_async_copy(buf.at[pl.ds(v0, ns)], o_hbm.at[pl.ds(n0, ns)], vsem.at[i]).wait()

    def kernel(*refs):
        pl.run_scoped(
            lambda *sems: body(*refs, *sems),
            pltpu.SemaphoreType.DMA((D,)),
            pltpu.SemaphoreType.DMA((D,)),
            pltpu.SemaphoreType.DMA((2 * RING,)),
            pltpu.SemaphoreType.DMA((TJ * RING,)),
            pltpu.SemaphoreType.DMA((2,)),
            pltpu.SemaphoreType.DMA((3,)))

    out = pl.pallas_call(
        kernel,
        in_specs=[pl.BlockSpec(memory_space=pl.ANY)] * 3,
        out_specs=pl.BlockSpec(memory_space=pl.ANY),
        out_shape=jax.ShapeDtypeStruct(x5.shape, x.dtype),
        scratch_shapes=[
            pltpu.VMEM(((RING + 1) * S, 2, SH, RS, W), x.dtype),
            pltpu.VMEM((2, 8, C // 8), g.dtype),
            pltpu.VMEM((16, C // 8), jnp.float32),
            pltpu.SMEM((16, C // 8), jnp.float32),
        ],
        compiler_params=pltpu.CompilerParams(
            vmem_limit_bytes=(RING + 2) * 8 * 1024 * 1024,
            disable_bounds_checks=True),
    )(x5, g2, b2)
    return out.reshape(x.shape)
```

```python
import jax
import jax.numpy as jnp
from jax import lax
import jax.experimental.pallas as pl
import jax.experimental.pallas.tpu as pltpu

EPS = 1e-5
NUM_GROUPS = 32

D = 16
DH = 10
RW_LEAD = 7
TJ = 4
TW = 2
RCW = 256
RPC = 128
WPC = (640, 640, 768)
AW = 256
HK = 2


def _shr(v, n):
    return v >> n if isinstance(v, int) else lax.shift_right_logical(v, jnp.int32(n))


def _and(v, m):
    return v & m if isinstance(v, int) else lax.bitwise_and(v, jnp.int32(m))


def _sel(p, vals):
    r = jnp.int32(vals[0])
    for i in range(1, len(vals)):
        r = jnp.where(p == i, jnp.int32(vals[i]), r)
    return r


@jax.jit
def pallas_standalone__groupnorm__prompt_kernel(
    x: jax.Array,
    g: jax.Array,
    b: jax.Array,
):
    B, C, H, W = x.shape
    assert (B, C, H, W) == (2, 1024, 32, 2048)
    G = NUM_GROUPS
    cpg = C // G
    RS = 8
    SPC = H // RS
    CPS = 8
    SH = CPS * SPC // 2
    NSTR = B * C // CPS
    S = 8
    SHIFT = 2
    V = NSTR // S - 1
    RING = 11
    RJ = W // RCW
    SPW = SH * RJ
    LSPW = SPW.bit_length() - 1
    LRJ = RJ.bit_length() - 1
    NSL = 3 * cpg * HK
    assert sum(WPC) == W
    wcols = [pl.ds(sum(WPC[:i]), WPC[i]) for i in range(len(WPC))]
    TCW = W // TJ
    n_el = cpg * H * W
    KR0 = (0, 11, 21)
    NWR = (11, 10, 10)
    GA = (0, 22, 42)
    LEAD = (4, 2, 2)
    NM = (18, 18, 20)
    KA = (0, 10, 20)
    NKW = (10, 10, 11)
    NP = 3
    assert all(m == 2 * (n - 1) for m, n in zip(NM, NKW))
    assert SPW % D == 0 and DH <= D and RW_LEAD < D
    assert all(SPW + l * NSL <= n * SPW - D for l, n in zip(LEAD, NWR)) and 2 * NSL >= SPW

    x5 = x.reshape(NSTR, 2, SH, RS, W)
    g2 = g.reshape(8, C // 8)
    b2 = b.reshape(8, C // 8)

    def body(x_hbm, g_hbm, b_hbm, o_hbm, buf, gb_bf, gb_f32, gb_s, lsem, hsem, wsem, tsem, vsem, psem):
        def pos_of(k):
            if isinstance(k, int):
                return k % RING
            return k - jnp.where(k >= 2 * RING, 2 * RING, jnp.where(k >= RING, RING, 0))

        def start(copies, priority):
            for c in copies:
                c.start(priority=priority)

        def wait(copies):
            for c in copies:
                c.wait()

        def rd(n0, v0, ns, u, sem):
            sl = _shr(u, LRJ)
            c0 = _and(u, RJ - 1) * RCW
            cs = pl.ds(c0 if isinstance(c0, int) else pl.multiple_of(c0, RCW), RCW)
            src = x_hbm.at[pl.ds(n0, ns), :, sl, :, cs]
            dst = buf.at[pl.ds(v0, ns), :, sl, :, cs]
            return [pltpu.make_async_copy(src.at[:, :, :, pl.ds(c, RPC)], dst.at[:, :, :, pl.ds(c, RPC)], sem)
                    for c in range(0, RCW, RPC)]

        def low(kr0, j):
            k = kr0 + _shr(j, LSPW)
            return rd(k * S + SHIFT, pos_of(k) * S, S - 1, _and(j, SPW - 1), lsem.at[_and(j, D - 1)])

        def high(kr0, j):
            k = kr0 + _shr(j, LSPW)
            return rd(k * S + SHIFT + S - 1, pos_of(k) * S + S - 1, 1, _and(j, SPW - 1),
                      hsem.at[_and(j, D - 1)])

        parts_v = ((V * S + SHIFT, RING * S, S - SHIFT), (0, RING * S + S - SHIFT, SHIFT))

        def low_v(j):
            return rd(*parts_v[0], j, lsem.at[_and(j, D - 1)])

        def high_v(j):
            return rd(*parts_v[1], j, hsem.at[_and(j, D - 1)])

        def wr(n0, v0, ns, half, sl, cs, sem):
            return pltpu.make_async_copy(buf.at[pl.ds(v0, ns), half, sl, :, cs],
                                         o_hbm.at[pl.ds(n0, ns), half, sl, :, cs], sem)

        def tail(k, t):
            pos = pos_of(k)
            return wr(k * S + SHIFT, pos * S, S, 1, SH - 1, pl.ds(t * TCW, TCW), tsem.at[TJ * pos + t])

        def issue_chunk(cid):
            k = _shr(cid, 1)
            half = _and(cid, 1)
            pos = pos_of(k)

            def slab(sl, c):
                for cs in wcols:
                    wr(k * S + SHIFT, pos * S, S, half, sl, cs, wsem.at[2 * pos + half]).start()
                return c
            lax.fori_loop(0, SH - half, slab, 0)

            @pl.when(half == 1)
            def _():
                for t in range(TJ):
                    tail(k, t).start()

        def wait_head(k):
            pos = pos_of(k)
            wr(k * S + SHIFT, pos * S, S, 0, pl.ds(0, SH), pl.ds(0, W), wsem.at[2 * pos]).wait()
            wr(k * S + SHIFT, pos * S, S, 1, pl.ds(0, SH - 1), pl.ds(0, W), wsem.at[2 * pos + 1]).wait()

        def tree(parts):
            while len(parts) > 1:
                parts = [parts[i] + parts[i + 1] for i in range(0, len(parts), 2)]
            return parts[0]

        def compute_group(gi, hook, cu):
            def vstream(s):
                n = _and(gi * 4 + s - SHIFT, NSTR - 1)
                k = _shr(n, 3)
                return jnp.where(k == V, RING, pos_of(k)) * S + _and(n, S - 1)
            nit = cpg // cu

            def refs(it):
                if cu == CPS:
                    base = buf.at[vstream(it)]
                    return [base.at[c // 4, pl.ds((c % 4) * SPC, SPC)] for c in range(cu)]
                assert cu == 1
                return [buf.at[vstream(_shr(it, 3)), _and(_shr(it, 2), 1), pl.ds(_and(it, 3) * SPC, SPC)]]

            def red(r, f, hk):
                outs = []
                for k in range(SPC):
                    if k % (SPC // HK) == 0:
                        hook(hk * HK + k // (SPC // HK))
                    v = f(r[k].astype(jnp.float32))
                    outs.append(tree([v[:, j * AW:(j + 1) * AW] for j in range(W // AW)]))
                return tree(outs)

            def p1(it, acc):
                for c, r in enumerate(refs(it)):
                    acc = acc + red(r, lambda v: v, it * cu + c)
                return acc
            acc = lax.fori_loop(0, nit, p1, jnp.zeros((RS, AW), jnp.float32))
            mu = jnp.sum(acc, keepdims=True) * (1.0 / n_el)

            def sq(v):
                d = v - mu
                return d * d

            def p2(it, acc):
                for c, r in enumerate(refs(it)):
                    acc = acc + red(r, sq, cpg + it * cu + c)
                return acc
            acc = lax.fori_loop(0, nit, p2, jnp.zeros((RS, AW), jnp.float32))
            var = jnp.sum(acc, keepdims=True) * (1.0 / n_el)
            rstd = lax.rsqrt(var + EPS)
            cb = _and(gi, G - 1) * cpg
            crow = _shr(cb, 7)
            ccol = _and(cb, 127)

            def p3(it, carry):
                for c, r in enumerate(refs(it)):
                    ch = ccol + it * cu + c
                    a = rstd * gb_s[crow, ch]
                    sh = gb_s[8 + crow, ch]
                    for hh in range(HK):
                        hook((2 * cpg + it * cu + c) * HK + hh)
                        rr = r.at[pl.ds(hh * (SPC // HK), SPC // HK)]
                        rr[...] = ((rr[...].astype(jnp.float32) - mu) * a + sh).astype(buf.dtype)
                return carry
            lax.fori_loop(0, nit, p3, 0)

        for j in range(DH):
            start(high_v(j), 0)
        for j in range(D):
            start(low_v(j), 1)
        cp_g = pltpu.make_async_copy(g_hbm, gb_bf.at[0], psem.at[0])
        cp_b = pltpu.make_async_copy(b_hbm, gb_bf.at[1], psem.at[1])
        cp_g.start()
        cp_b.start()

        def pace_v(j, c):
            wait(low_v(j))
            wait(high_v(j))
            start(high_v(j + DH), 0)
            start(low_v(j + D), 1)
            return c
        lax.fori_loop(0, 16, pace_v, 0)
        cp_g.wait()
        cp_b.wait()
        gb_f32[0:8, :] = gb_bf[0].astype(jnp.float32)
        gb_f32[8:16, :] = gb_bf[1].astype(jnp.float32)
        cp_s = pltpu.make_async_copy(gb_f32, gb_s, psem.at[2])
        cp_s.start()
        lax.fori_loop(16, SPW - D, pace_v, 0)
        cp_s.wait()
        for j in range(SPW - D, SPW):
            wait(low_v(j))
            wait(high_v(j))
            start(high_v(j + DH) if j + DH < SPW else high(0, j + DH - SPW), 0)
            start(low(0, j + D - SPW), 1)

        def phase(p, carry):
            kr0 = _sel(p, KR0)
            nsteps = _sel(p, NWR) * SPW
            ga = _sel(p, GA)
            lead = _sel(p, LEAD)
            ka = _sel(p, KA)

            def pace(j):
                wait(low(kr0, j))
                wait(high(kr0, j))
                start(high(kr0, j + DH), 0)
                start(low(kr0, j + D), 1)

            def pace_loop(lo, hi):
                def step(j, c):
                    pace(j)
                    return c
                lax.fori_loop(lo, hi, step, 0)

            pace_loop(0, SPW)

            def lead_group(q, c):
                compute_group(ga + q, lambda k: pace(SPW + q * NSL + k), 1)
                return c
            lax.fori_loop(0, lead, lead_group, 0)
            pace_loop(SPW + lead * NSL, nsteps - D)
            for t in range(D):
                j = nsteps - D + t
                wait(low(kr0, j))
                wait(high(kr0, j))
                if t + DH < D:
                    start(high(kr0, j + DH), 0)
                if t == D - 1 - RW_LEAD:
                    issue_chunk(2 * ka)
            issue_chunk(2 * ka + 1)

            def write_group(m, c):
                compute_group(ga + lead + m, lambda k: None, CPS)
                issue_chunk(2 * ka + 2 + m)

                @pl.when(_and(m, 1) == 1)
                def _():
                    k = ka + _shr(m, 1)
                    wait_head(k)
                    for t in range(TJ):
                        tail(k, t).wait()
                return c
            lax.fori_loop(0, _sel(p, NM), write_group, 0)

            @pl.when(p == NP - 1)
            def _():
                for half in range(2):
                    def slab_v(sl, c):
                        for cs in wcols:
                            for i, (n0, v0, ns) in enumerate(parts_v):
                                wr(n0, v0, ns, half, sl, cs, vsem.at[i]).start()
                        return c
                    lax.fori_loop(0, SH, slab_v, 0)

            k_last = ka + _sel(p, NKW) - 1
            wait_head(k_last)
            for t in range(TW):
                tail(k_last, t).wait()

            @pl.when(p < NP - 1)
            def _():
                kr_next = kr0 + _sel(p, NWR)
                for j in range(DH):
                    start(high(kr_next, j), 0)
                for j in range(D):
                    start(low(kr_next, j), 1)
            for t in range(TW, TJ):
                tail(k_last, t).wait()
            return carry
        lax.fori_loop(0, NP, phase, 0)
        for i, (n0, v0, ns) in enumerate(parts_v):
            pltpu.make_async_copy(buf.at[pl.ds(v0, ns)], o_hbm.at[pl.ds(n0, ns)], vsem.at[i]).wait()

    def kernel(*refs):
        pl.run_scoped(
            lambda *sems: body(*refs, *sems),
            pltpu.SemaphoreType.DMA((D,)),
            pltpu.SemaphoreType.DMA((D,)),
            pltpu.SemaphoreType.DMA((2 * RING,)),
            pltpu.SemaphoreType.DMA((TJ * RING,)),
            pltpu.SemaphoreType.DMA((2,)),
            pltpu.SemaphoreType.DMA((3,)))

    out = pl.pallas_call(
        kernel,
        in_specs=[pl.BlockSpec(memory_space=pl.ANY)] * 3,
        out_specs=pl.BlockSpec(memory_space=pl.ANY),
        out_shape=jax.ShapeDtypeStruct(x5.shape, x.dtype),
        scratch_shapes=[
            pltpu.VMEM(((RING + 1) * S, 2, SH, RS, W), x.dtype),
            pltpu.VMEM((2, 8, C // 8), g.dtype),
            pltpu.VMEM((16, C // 8), jnp.float32),
            pltpu.SMEM((16, C // 8), jnp.float32),
        ],
        compiler_params=pltpu.CompilerParams(
            vmem_limit_bytes=(RING + 2) * 8 * 1024 * 1024,
            disable_bounds_checks=True),
    )(x5, g2, b2)
    return out.reshape(x.shape)
```
